```python
import os as _os
_os.environ.setdefault("JAX_PLATFORMS", "cpu")
import jax
import jax.numpy as jnp

def _softmax(x, axis=-1):
    return jax.nn.softmax(x, axis=axis)
def _gelu(x):
    return jax.nn.gelu(x, approximate=True)
def _silu(x):
    return jax.nn.silu(x)
def _sigmoid(x):
    return jax.nn.sigmoid(x)
def _layernorm(x, axis=-1, eps=1e-5):
    m = jnp.mean(x, axis=axis, keepdims=True)
    v = jnp.var(x, axis=axis, keepdims=True)
    return (x - m) / jnp.sqrt(v + eps)
def _scatter_add(tgt, idx, src, axis=0):
    return tgt.at[idx].add(src)
def _segment_sum(src, seg, n):
    return jax.ops.segment_sum(src, seg, n)
class _Rng:
    def __init__(self, key):
        self._k = key
    def _next(self):
        self._k, sub = jax.random.split(self._k)
        return sub
    def normal(self, shape):
        return jax.random.normal(self._next(), shape, dtype=jnp.bfloat16)
    def randint(self, lo, hi, shape):
        return jax.random.randint(self._next(), shape, lo, hi, dtype=jnp.int32)
    def uniform(self, shape, lo=0.0, hi=1.0):
        return jax.random.uniform(self._next(), shape, jnp.bfloat16, lo, hi)
    def permutation(self, n):
        return jax.random.permutation(self._next(), n)


kernel_name = 'standalone__gqa_softmax__near_ridge'

def setup_inputs():
    _rng = _Rng(jax.random.key(int.from_bytes(__import__("os").urandom(4), "little")))
    _w = (lambda a: (lambda t: t.astype(jnp.bfloat16) if jnp.issubdtype(t.dtype, jnp.floating) else t)(jnp.asarray(a)))
    B, Hq, Hkv, Sq, Sk, D = 16, 32, 32, 368, 512, 192
    return {
        "q": _w((lambda *s: _rng.normal(s) * 0.4)(B, Hq, Sq, D)),
        "k": _w((lambda *s: _rng.normal(s) * 0.4)(B, Hkv, Sk, D)),
        "v": _w((lambda *s: _rng.normal(s) * 0.05)(B, Hkv, Sk, D)),
    }

def reference(q, k, v):
    B, Hq, Sq, D = q.shape
    Hkv = k.shape[1]
    rep = Hq // Hkv
    k = jnp.repeat(k, rep, axis=1)
    v = jnp.repeat(v, rep, axis=1)
    scale = D ** -0.5
    scores = jnp.einsum("bhqd,bhkd->bhqk", q, k) * scale
    p = _softmax(scores, axis=-1)
    return jnp.einsum("bhqk,bhkd->bhqd", p, v)
```

```python
import math

import jax
import jax.numpy as jnp
from jax import lax
import jax.experimental.pallas as pl
import jax.experimental.pallas.tpu as pltpu

_U = 4


@jax.jit
def pallas_standalone__gqa_softmax__near_ridge_kernel(
    q: jax.Array,
    k: jax.Array,
    v: jax.Array,
):
    B, H, Sq, D = q.shape
    Sk = k.shape[2]
    assert k.shape == v.shape == (B, H, Sk, D)
    N = B * H
    U = _U
    steps = N // U
    R = 4 * U
    c = (D ** -0.5) * math.log2(math.e)
    f32, bf16 = jnp.float32, jnp.bfloat16

    def softmax(s):
        m = jnp.max(s, axis=1, keepdims=True)
        p = jnp.exp2((s - m) * c)
        l = jnp.sum(p, axis=1, keepdims=True)
        return (p * (1.0 / l)).astype(bf16)

    def kernel(q_hbm, k_hbm, v_hbm, o_hbm, qb, kb, vb, ob, t_scr, s_scr, sems):
        def rd(i):
            slot = (i % 4) * U
            return [
                pltpu.make_async_copy(src.at[pl.ds(i * U, U)], dst.at[pl.ds(slot, U)], sems.at[j, i % 4])
                for j, (src, dst) in enumerate(((q_hbm, qb), (k_hbm, kb), (v_hbm, vb)))
            ]

        def wr(i):
            return pltpu.make_async_copy(
                ob.at[pl.ds((i % 2) * U, U)], o_hbm.at[pl.ds(i * U, U)], sems.at[3, i % 2])

        for i in range(3):
            for cp in rd(i):
                cp.start()
        for cp in rd(0):
            cp.wait()
        s_scr[...] = jnp.dot(qb[0].T, kb[0], preferred_element_type=f32)
        t_scr[...] = qb[1].T

        def body(i, _):
            @pl.when(i + 1 < steps)
            def _():
                for cp in rd(i + 1):
                    cp.wait()

            @pl.when(i + 3 < steps)
            def _():
                for cp in rd(i + 3):
                    cp.start()

            @pl.when(i >= 2)
            def _():
                wr(i - 2).wait()

            h0 = i * U
            slot = lambda h: jnp.minimum(h, N - 1) % R
            s = s_scr[...]
            t = t_scr[...]
            for u in range(U):
                s_next = jnp.dot(t, kb[slot(h0 + u + 1)], preferred_element_type=f32)
                t = qb[slot(h0 + u + 2)].T
                p = softmax(s)
                ob[(i % 2) * U + u] = lax.dot_general(
                    vb[slot(h0 + u)], p, (((1,), (1,)), ((), ())), preferred_element_type=f32).astype(bf16)
                s = s_next
            s_scr[...] = s
            t_scr[...] = t
            wr(i).start()

        lax.fori_loop(0, steps, body, None)
        wr(steps - 2).wait()
        wr(steps - 1).wait()

    qT = jnp.swapaxes(q, 2, 3).reshape(N, D, Sq)
    kT = jnp.swapaxes(k, 2, 3).reshape(N, D, Sk)
    vT = jnp.swapaxes(v, 2, 3).reshape(N, D, Sk)
    oT = pl.pallas_call(
        kernel,
        in_specs=[pl.BlockSpec(memory_space=pl.ANY)] * 3,
        out_specs=pl.BlockSpec(memory_space=pl.ANY),
        out_shape=jax.ShapeDtypeStruct((N, D, Sq), bf16),
        scratch_shapes=[
            pltpu.VMEM((R, D, Sq), bf16),
            pltpu.VMEM((R, D, Sk), bf16),
            pltpu.VMEM((R, D, Sk), bf16),
            pltpu.VMEM((2 * U, D, Sq), bf16),
            pltpu.VMEM((Sq, D), bf16),
            pltpu.VMEM((Sq, Sk), f32),
            pltpu.SemaphoreType.DMA((4, 4)),
        ],
        compiler_params=pltpu.CompilerParams(vmem_limit_bytes=64 * 2**20),
    )(qT, kT, vT)
    return jnp.swapaxes(oT.reshape(B, H, D, Sq), 2, 3)
```

```python
import math

import jax
import jax.numpy as jnp
from jax import lax
import jax.experimental.pallas as pl
import jax.experimental.pallas.tpu as pltpu

_U = 8
_RING = 10
_WRITE_ROWS = 16

_READ1_END = 35 / 64
_WRITE1_AT = 215 / 512
_READ2_AT = 263 / 512
_WRITE2_AT = 447 / 512


@jax.jit
def pallas_standalone__gqa_softmax__near_ridge_kernel(
    q: jax.Array,
    k: jax.Array,
    v: jax.Array,
):
    B, H, Sq, D = q.shape
    Sk = k.shape[2]
    assert k.shape == v.shape == (B, H, Sk, D), "one kv head per query head"
    N, U = B * H, _U
    steps = N // U
    assert steps * U == N and steps > _RING
    f32, bf16 = jnp.float32, jnp.bfloat16
    exp2_scale = (D**-0.5) * math.log2(math.e)
    q_tiles = [(r, min(128, Sq - r)) for r in range(0, Sq, 128)]
    k_halves = [pl.ds(0, Sk // 2), pl.ds(Sk // 2, Sk // 2)]

    read1_end = round(_READ1_END * steps)
    write1_at, read2_at, write2_at = (
        round(x * N) for x in (_WRITE1_AT, _READ2_AT, _WRITE2_AT)
    )
    assert read2_at < read1_end * U
    read_slots = (read2_at % U, (read2_at + U // 2) % U)
    write_at = [write1_at, *range(write2_at, N - U, 2 * U), N - U]
    writes = list(zip([0] + write_at, write_at))

    def softmax(s):
        m = jnp.max(s, axis=1, keepdims=True)
        p = jnp.exp2((s - m) * exp2_scale)
        l = jnp.sum(p, axis=1, keepdims=True)
        r = pltpu.reciprocal(l, approx=True)
        r = r * (2.0 - l * r)
        return (p * r).astype(bf16)

    def kernel(q_hbm, k_hbm, v_hbm, o_hbm,
               q_buf, k_buf, v_buf, o_buf, q_first, k_first, qt_carry, s_carry,
               read_sem, first_sem, write_sem):

        def reads(c, slot):
            copies = []
            for j, (src, dst, ahead) in enumerate(
                ((q_hbm, q_buf, 2), (k_hbm, k_buf, 1), (v_hbm, v_buf, 0))
            ):
                n = U
                if ahead and not isinstance(c, int):
                    n = jnp.where(c == steps - 1, U - ahead, U)
                copies.append(pltpu.make_async_copy(
                    src.at[pl.ds(c * U + ahead, n)],
                    dst.at[slot, pl.ds(0, n)],
                    read_sem.at[j, slot]))
            return copies

        first = [
            pltpu.make_async_copy(q_hbm.at[pl.ds(0, 2)], q_first, first_sem.at[0]),
            pltpu.make_async_copy(k_hbm.at[0], k_first, first_sem.at[1]),
        ]
        for copy in first + reads(0, 0):
            copy.start()
        for copy in first:
            copy.wait()
        s_carry[...] = jnp.dot(q_first[0].T, k_first[...], preferred_element_type=f32)
        qt_carry[...] = pltpu.bitcast(q_first[1].T, jnp.uint32)

        def body(i, carry):
            slot, fetch, fetch_slot = carry

            @pl.when(i == 0)
            def _():
                for copy in reads(1, 1):
                    copy.start()

            for copy in reads(i, slot):
                copy.wait()

            qt = pltpu.bitcast(qt_carry[...], bf16)
            s = None
            for u in range(U):
                h = i * U + u
                if u in read_slots:
                    limit = jnp.where(h < read2_at, read1_end, steps)
                    go = fetch < jnp.minimum(i + _RING, limit)

                    @pl.when(go)
                    def _():
                        for copy in reads(fetch, fetch_slot):
                            copy.start()

                    fetch = jnp.where(go, fetch + 1, fetch)
                    fetch_slot = jnp.where(go, fetch_slot + 1, fetch_slot)
                    fetch_slot = jnp.where(fetch_slot == _RING, 0, fetch_slot)

                if any(at % U == u for at in write_at):
                    h0 = n = jnp.int32(0)
                    for lo, at in writes:
                        if at % U == u:
                            h0 = jnp.where(h == at, lo, h0)
                            n = jnp.where(h == at, at - lo, n)

                    @pl.when(n > 0)
                    def _():
                        for r in range(0, D, _WRITE_ROWS):
                            part = (pl.ds(h0, n), pl.ds(r, _WRITE_ROWS))
                            pltpu.make_async_copy(
                                o_buf.at[part], o_hbm.at[part], write_sem).start()

                def scores(half):
                    return jnp.dot(qt, k_buf[slot, u, :, k_halves[half]],
                                   preferred_element_type=f32)

                def output(tile):
                    r, n = q_tiles[tile]
                    if u == 0:
                        s_tile = s_carry[pl.ds(r, n), :]
                    else:
                        s_tile = jnp.concatenate([x[r:r + n] for x in s], axis=1)
                    o_buf[h, :, pl.ds(r, n)] = lax.dot_general(
                        v_buf[slot, u], softmax(s_tile), (((1,), (1,)), ((), ())),
                        preferred_element_type=f32).astype(bf16)

                qt_next = q_buf[slot, u].T
                before = len(q_tiles) - 1 if u < U - 1 else 0
                s_lo = scores(0)
                for tile in range(before):
                    output(tile)
                s_hi = scores(1)
                for tile in range(before, len(q_tiles)):
                    output(tile)
                qt, s = qt_next, (s_lo, s_hi)

            for half in range(2):
                s_carry[:, k_halves[half]] = s[half]
            qt_carry[...] = pltpu.bitcast(qt, jnp.uint32)
            return jnp.where(slot == _RING - 1, 0, slot + 1), fetch, fetch_slot

        lax.fori_loop(0, steps, body, (jnp.int32(0), jnp.int32(2), jnp.int32(2)))
        last = pl.ds(N - U, U)
        pltpu.make_async_copy(o_buf.at[last], o_hbm.at[last], write_sem).start()
        pltpu.make_async_copy(o_buf, o_buf, write_sem).wait()

    o_t = pl.pallas_call(
        kernel,
        in_specs=[pl.BlockSpec(memory_space=pl.ANY)] * 3,
        out_specs=pl.BlockSpec(memory_space=pl.ANY),
        out_shape=jax.ShapeDtypeStruct((N, D, Sq), bf16),
        scratch_shapes=[
            pltpu.VMEM((_RING, U, D, Sq), bf16),
            pltpu.VMEM((_RING, U, D, Sk), bf16),
            pltpu.VMEM((_RING, U, D, Sk), bf16),
            pltpu.VMEM((N, D, Sq), bf16),
            pltpu.VMEM((2, D, Sq), bf16),
            pltpu.VMEM((D, Sk), bf16),
            pltpu.VMEM((Sq // 2, D), jnp.uint32),
            pltpu.VMEM((Sq, Sk), f32),
            pltpu.SemaphoreType.DMA((3, _RING)),
            pltpu.SemaphoreType.DMA((2,)),
            pltpu.SemaphoreType.DMA(()),
        ],
        compiler_params=pltpu.CompilerParams(
            vmem_limit_bytes=126 * 2**20, disable_bounds_checks=True),
    )(
        jnp.swapaxes(q, 2, 3).reshape(N, D, Sq),
        jnp.swapaxes(k, 2, 3).reshape(N, D, Sk),
        jnp.swapaxes(v, 2, 3).reshape(N, D, Sk),
    )
    return jnp.swapaxes(o_t.reshape(B, H, D, Sq), 2, 3)
```

```python
import functools
import math

import jax
import jax.numpy as jnp
from jax import lax
import jax.experimental.pallas as pl
import jax.experimental.pallas.tpu as pltpu

_UNROLL = 32
_RING = 128

_FETCH_AHEAD = 3
_FETCH_RATE = 41
_Q_PIECES = 3
_WRITE_HEADS, _WRITE_ROWS = 31, 8
_WRITE_TAIL = 16
_WRITE_RATE = 115
_WRITE_DELAY = 1425


def _due(slot, slots, items):
    return range(slot * items // slots, (slot + 1) * items // slots)


def _check_pacing(n, parts):
    total = (n - _WRITE_TAIL) // _WRITE_HEADS * parts
    for h in range(n):
        assert _FETCH_AHEAD + h * _FETCH_RATE // _UNROLL > h
        assert min(_FETCH_AHEAD + pl.cdiv((h + 1) * _FETCH_RATE, _UNROLL), n) < h + _RING
        written = (h + 1) * _WRITE_RATE // _UNROLL - _WRITE_DELAY
        assert pl.cdiv(min(written, total), parts) * _WRITE_HEADS <= h
    assert written >= total


@jax.jit
def pallas_standalone__gqa_softmax__near_ridge_kernel(
    q: jax.Array,
    k: jax.Array,
    v: jax.Array,
):
    B, H, Sq, D = q.shape
    Sk = k.shape[2]
    assert k.shape == v.shape == (B, H, Sk, D), "one kv head per query head"
    N, U = B * H, _UNROLL
    steps = N // U
    assert N % U == 0 and _RING % U == 0 and (N - _WRITE_TAIL) % _WRITE_HEADS == 0
    assert 256 < Sq <= 384 and D % (16 * _Q_PIECES) == 0
    f32, bf16 = jnp.float32, jnp.bfloat16
    exp2_scale = (D**-0.5) * math.log2(math.e)
    q_tiles = [(r, min(128, Sq - r)) for r in range(0, Sq, 128)]
    k_halves = [pl.ds(0, Sk // 2), pl.ds(Sk // 2, Sk // 2)]
    q_rows = D // _Q_PIECES
    write_parts = D // _WRITE_ROWS
    tail = N - _WRITE_TAIL
    _check_pacing(N, write_parts)

    def softmax(s):
        m = jnp.max(s, axis=1, keepdims=True)
        p = jnp.exp2((s - m) * exp2_scale)
        l = jnp.sum(p, axis=1, keepdims=True)
        r = pltpu.reciprocal(l, approx=True)
        r = r * (2.0 - l * r)
        return (p * r).astype(bf16)

    def kernel(q_hbm, k_hbm, v_hbm, o_hbm,
               k_buf, v_buf, qo_buf, qt_carry, s_carry,
               read_sem, first_sem, write_sem):
        def q_copy(c, piece):
            rows = pl.ds(piece * q_rows, q_rows)
            return pltpu.make_async_copy(
                q_hbm.at[c + 3, rows], qo_buf.at[c + 3, rows], read_sem.at[c & (_RING - 1)])

        def k_copy(c):
            slot = c & (_RING - 1)
            return pltpu.make_async_copy(k_hbm.at[c + 2], k_buf.at[slot], read_sem.at[slot])

        def v_copy(c, piece):
            slot, rows = c & (_RING - 1), pl.ds(piece * (D // 2), D // 2)
            return pltpu.make_async_copy(
                v_hbm.at[c + 1, rows], v_buf.at[slot, rows], read_sem.at[slot])

        v_copies = [(functools.partial(v_copy, piece=p), 1) for p in range(2)]
        q_copies = [(functools.partial(q_copy, piece=p), 3) for p in range(_Q_PIECES)]
        set_copies = v_copies + [(k_copy, 2)] + q_copies

        def o_copy(*index):
            return pltpu.make_async_copy(qo_buf.at[index], o_hbm.at[index], write_sem)

        first = [
            pltpu.make_async_copy(src, dst, first_sem.at[j])
            for j, (src, dst) in enumerate((
                (q_hbm.at[0], qo_buf.at[0]), (k_hbm.at[0], k_buf.at[_RING - 2]),
                (q_hbm.at[1], qo_buf.at[1]), (k_hbm.at[1], k_buf.at[_RING - 1]),
                (q_hbm.at[2], qo_buf.at[2]), (v_hbm.at[0], v_buf.at[_RING - 1]),
            ))
        ]
        for copy in first:
            copy.start()
        for c in range(_FETCH_AHEAD):
            for copy, _ in set_copies:
                copy(c).start(priority=1)
        first[0].wait()
        qt = qo_buf[0].T
        first[1].wait()
        s = jnp.dot(qt, k_buf[_RING - 2], preferred_element_type=f32)
        first[2].wait()
        qt_carry[...] = pltpu.bitcast(qo_buf[1].T, jnp.uint32)
        s_carry[...] = s
        for copy in first[3:]:
            copy.wait()

        def body(i, _):
            fetched = _FETCH_AHEAD + i * _FETCH_RATE
            written = i * _WRITE_RATE - _WRITE_DELAY
            ring_base = (i * U) & (_RING - 1)
            qt = pltpu.bitcast(qt_carry[...], bf16)
            s = None
            for u in range(U):
                h = i * U + u
                slot = ring_base + (u - 1) if u else (h - 1) & (_RING - 1)

                def fetch(copy, ahead):
                    for item in _due(u, U, _FETCH_RATE):
                        c = fetched + item
                        pl.when(c + ahead < N)(lambda: copy(c).start(priority=1))

                def pulse(j):
                    for item in _due(4 * u + j, 4 * U, _FETCH_RATE * _Q_PIECES):
                        c = fetched + item // _Q_PIECES
                        pl.when(c + 3 < N)(lambda: q_copy(c, item % _Q_PIECES).start())
                    for item in _due(4 * u + j, 4 * U, _WRITE_RATE):
                        w = written + item

                        @pl.when(jnp.logical_and(w >= 0, w < tail // _WRITE_HEADS * write_parts))
                        def _():
                            group = lax.div(w, write_parts)
                            row = (w - group * write_parts) * _WRITE_ROWS
                            o_copy(pl.ds(group * _WRITE_HEADS, _WRITE_HEADS),
                                   pl.ds(pl.multiple_of(row, _WRITE_ROWS), _WRITE_ROWS)).start()

                def await_next_inputs():
                    for copy, ahead in set_copies:
                        if u + ahead < U:
                            copy(h).wait()
                        else:
                            pl.when(i < steps - 1)(lambda: copy(h).wait())

                def scores(half):
                    return jnp.dot(qt, k_buf[slot, :, k_halves[half]],
                                   preferred_element_type=f32)

                def attend(tile):
                    r, n = q_tiles[tile]
                    if u == 0:
                        s_tile = s_carry[pl.ds(r, n), :]
                    else:
                        s_tile = jnp.concatenate([x[r:r + n] for x in s], axis=1)
                    return lax.dot_general(
                        v_buf[slot], softmax(s_tile), (((1,), (1,)), ((), ())),
                        preferred_element_type=f32).astype(bf16)

                def store(tile, o):
                    qo_buf[h, :, pl.ds(*q_tiles[tile])] = o

                last = u == U - 1
                pulse(0)
                pl.when(h > tail)(lambda: o_copy(h - 1).start())
                s_lo = scores(0)
                if last:
                    s_hi = scores(1)
                o0 = attend(0)
                fetch(*v_copies[0])
                pulse(1)
                fetch(*v_copies[1])
                o1 = attend(1)
                qt_next = qo_buf[h + 2 if u + 2 < U else jnp.minimum(h + 2, N - 1)].T
                store(0, o0)
                pulse(2)
                store(1, o1)
                if not last:
                    s_hi = scores(1)
                fetch(k_copy, 2)
                o2 = attend(2)
                await_next_inputs()
                pulse(3)
                store(2, o2)
                qt, s = qt_next, (s_lo, s_hi)

            for half in range(2):
                s_carry[:, k_halves[half]] = s[half]
            qt_carry[...] = pltpu.bitcast(qt, jnp.uint32)

        lax.fori_loop(0, steps, body, None)
        o_copy(N - 1).start()
        pltpu.make_async_copy(qo_buf, o_hbm, write_sem).wait()

    o_t = pl.pallas_call(
        kernel,
        in_specs=[pl.BlockSpec(memory_space=pl.ANY)] * 3,
        out_specs=pl.BlockSpec(memory_space=pl.ANY),
        out_shape=jax.ShapeDtypeStruct((N, D, Sq), bf16),
        scratch_shapes=[
            pltpu.VMEM((_RING, D, Sk), bf16),
            pltpu.VMEM((_RING, D, Sk), bf16),
            pltpu.VMEM((N, D, Sq), bf16),
            pltpu.VMEM((Sq // 2, D), jnp.uint32),
            pltpu.VMEM((Sq, Sk), f32),
            pltpu.SemaphoreType.DMA((_RING,)),
            pltpu.SemaphoreType.DMA((6,)),
            pltpu.SemaphoreType.DMA(()),
        ],
        compiler_params=pltpu.CompilerParams(
            vmem_limit_bytes=127 * 2**20,
            disable_bounds_checks=True,
            disable_semaphore_checks=True,
            flags={"XLA_TPU_RESCHEDULE_DMA_DONES": True},
        ),
    )(
        jnp.swapaxes(q, 2, 3).reshape(N, D, Sq),
        jnp.swapaxes(k, 2, 3).reshape(N, D, Sk),
        jnp.swapaxes(v, 2, 3).reshape(N, D, Sk),
    )
    return jnp.swapaxes(o_t.reshape(B, H, D, Sq), 2, 3)
```
